```python
import jax
import jax.numpy as jnp

def _softmax(x, axis=-1):
    return jax.nn.softmax(x, axis=axis)
def _gelu(x):
    return jax.nn.gelu(x, approximate=True)
def _silu(x):
    return jax.nn.silu(x)
def _sigmoid(x):
    return jax.nn.sigmoid(x)
def _layernorm(x, axis=-1, eps=1e-5):
    m = jnp.mean(x, axis=axis, keepdims=True)
    v = jnp.var(x, axis=axis, keepdims=True)
    return (x - m) / jnp.sqrt(v + eps)
def _scatter_add(tgt, idx, src, axis=0):
    return tgt.at[idx].add(src)
def _segment_sum(src, seg, n):
    return jax.ops.segment_sum(src, seg, n)
class _Rng:
    def __init__(self, key):
        self._k = key
    def _next(self):
        self._k, sub = jax.random.split(self._k)
        return sub
    def normal(self, shape):
        return jax.random.normal(self._next(), shape, dtype=jnp.bfloat16)
    def randint(self, lo, hi, shape):
        return jax.random.randint(self._next(), shape, lo, hi, dtype=jnp.int32)
    def uniform(self, shape, lo=0.0, hi=1.0):
        return jax.random.uniform(self._next(), shape, jnp.bfloat16, lo, hi)
    def permutation(self, n):
        return jax.random.permutation(self._next(), n)


kernel_name = 'standalone__cross_network_dcn_v2__recsys'

def setup_inputs():
    _rng = _Rng(jax.random.key(int.from_bytes(__import__("os").urandom(4), "little")))
    _w = (lambda a: (lambda t: t.astype(jnp.bfloat16) if jnp.issubdtype(t.dtype, jnp.floating) else t)(jnp.asarray(a)))
    B, F, D, L = 16384, 100, 16, 3
    Din = min(F * D, 512)
    R = max(Din // 4, 2)
    sc = Din ** -0.5
    return {
        "x0": _w((lambda *s: _rng.normal(s) * 0.05)(B, Din)),
        "U":  _w((lambda *s: _rng.normal(s) * 0.05)(L, Din, R) * sc),
        "V":  _w((lambda *s: _rng.normal(s) * 0.05)(L, R, Din) * sc),
        "bs": _w((lambda *s: _rng.normal(s) * 0.05)(L, Din)),
    }

def reference(x0, U, V, bs):
    x = x0
    for l in range(U.shape[0]):
        h = jnp.einsum('rd,bd->br', V[l], x)
        h = jnp.einsum('dr,br->bd', U[l], h)
        x = x0 * (h + bs[l]) + x
    return x
```

```python
import jax
import jax.numpy as jnp
from jax import lax
import jax.experimental.pallas as pl
import jax.experimental.pallas.tpu as pltpu

_BM = 1024
_SUB = 256


def _dcn_kernel(x0_ref, u_ref, v_ref, b_ref, o_ref):
    n_layers = u_ref.shape[0]
    nt = (((1,), (1,)), ((), ()))
    for c in range(_BM // _SUB):
        rows = pl.ds(c * _SUB, _SUB)
        x0 = x0_ref[rows, :]
        x0f = x0.astype(jnp.float32)
        x = x0
        for l in range(n_layers):
            h = lax.dot_general(x, v_ref[l], nt, preferred_element_type=jnp.float32)
            h = h.astype(jnp.bfloat16)
            y = lax.dot_general(h, u_ref[l], nt, preferred_element_type=jnp.float32)
            b = b_ref[l:l + 1, :].astype(jnp.float32)
            x = (x0f * (y + b) + x.astype(jnp.float32)).astype(jnp.bfloat16)
        o_ref[rows, :] = x


@jax.jit
def pallas_standalone__cross_network_dcn_v2__recsys_kernel(x0, U, V, bs):
    B, D = x0.shape
    L, _, R = U.shape
    return pl.pallas_call(
        _dcn_kernel,
        grid=(B // _BM,),
        in_specs=[
            pl.BlockSpec((_BM, D), lambda i: (i, 0)),
            pl.BlockSpec((L, D, R), lambda i: (0, 0, 0)),
            pl.BlockSpec((L, R, D), lambda i: (0, 0, 0)),
            pl.BlockSpec((L, D), lambda i: (0, 0)),
        ],
        out_specs=pl.BlockSpec((_BM, D), lambda i: (i, 0)),
        out_shape=jax.ShapeDtypeStruct((B, D), x0.dtype),
        compiler_params=pltpu.CompilerParams(dimension_semantics=("parallel",)),
    )(x0, U, V, bs)
```

```python
import jax
import jax.numpy as jnp
from jax import lax
import jax.experimental.pallas as pl
import jax.experimental.pallas.tpu as pltpu

_PROLOGUE = ((512,), (512,) * 2, (512,) * 5)
_LOOP_TILES = (512,) * 7 + (256, 256)
_LAST_SPLIT = 2

_NT = (((1,), (1,)), ((), ()))


def _offsets(sizes):
    out, start = [], 0
    for size in sizes:
        out.append((start, size))
        start += size
    return out


def _dcn_kernel(x_hbm, u_hbm, v_hbm, b_hbm, o_hbm, x_loop, *scratch):
    n_layers = u_hbm.shape[0]
    n_iter, loop_rows, _ = x_loop.shape
    n_pro = len(_PROLOGUE)
    chunks = _offsets([sum(tiles) for tiles in _PROLOGUE])
    pro_rows = sum(size for _, size in chunks)

    x_pro = scratch[:n_pro]
    u_buf = scratch[n_pro:n_pro + n_layers]
    v_buf = scratch[n_pro + n_layers:n_pro + 2 * n_layers]
    b_buf, in_sem, out_sem = scratch[n_pro + 2 * n_layers:]

    def pro_copy(c):
        start, size = chunks[c]
        sem = in_sem.at[0 if c == 0 else 2 + c % 2]
        return pltpu.make_async_copy(x_hbm.at[pl.ds(start, size)], x_pro[c], sem)

    def loop_copy(i):
        src = x_hbm.at[pl.ds(pro_rows + i * loop_rows, loop_rows)]
        return pltpu.make_async_copy(src, x_loop.at[i], in_sem.at[2 + (n_pro + i) % 2])

    def weight_copies(l):
        sem = in_sem.at[min(l, 1)]
        return [pltpu.make_async_copy(v_hbm.at[l], v_buf[l], sem),
                pltpu.make_async_copy(u_hbm.at[l], u_buf[l], sem)]

    def out_copy(src, start):
        return pltpu.make_async_copy(src, o_hbm.at[pl.ds(start, src.shape[0])], out_sem)

    def layer(l, x, x0_f32):
        h = lax.dot_general(x, v_buf[l][...], _NT, preferred_element_type=jnp.float32)
        h = lax.dot_general(h.astype(x.dtype), u_buf[l][...], _NT,
                            preferred_element_type=jnp.float32)
        bias = b_buf[l:l + 1, :].astype(jnp.float32)
        return (x0_f32 * (h + bias) + x.astype(jnp.float32)).astype(x.dtype)

    first = weight_copies(0) + [pltpu.make_async_copy(b_hbm, b_buf, in_sem.at[0]),
                                pro_copy(0)]
    rest = [c for l in range(1, n_layers) for c in weight_copies(l)]
    for copy in first + rest:
        copy.start()
    pro_copy(1).start(priority=1)

    pending = []
    for c, tiles in enumerate(_PROLOGUE):
        if c == 0:
            for copy in first:
                copy.wait()
        else:
            pro_copy(c).wait()
        if c + 2 < n_pro:
            pro_copy(c + 2).start(priority=1)
        elif c + 2 == n_pro:
            loop_copy(0).start(priority=1)
        for start, size in _offsets(tiles):
            tile = x_pro[c].at[pl.ds(start, size)]
            x = tile[...]
            x0_f32 = x.astype(jnp.float32)
            for l in range(n_layers):
                if c == 0 and start == 0 and l == 1:
                    for copy in rest:
                        copy.wait()
                x = layer(l, x, x0_f32)
            tile[...] = x
            pending.append(out_copy(tile, chunks[c][0] + start))
            if c == n_pro - 1:
                for copy in pending:
                    copy.start()
                pending = []

    def body(i, carry):
        loop_copy(i).wait()

        @pl.when(i + 1 < n_iter)
        def _():
            loop_copy(i + 1).start(priority=1)

        for k, (start, size) in enumerate(_offsets(_LOOP_TILES)):
            x = x_loop[i, pl.ds(start, size), :]
            x0_f32 = x.astype(jnp.float32)
            for l in range(n_layers):
                x = layer(l, x, x0_f32)
            pieces = _LAST_SPLIT if k == len(_LOOP_TILES) - 1 else 1
            rows = size // pieces
            for p in range(pieces):
                piece = x_loop.at[i, pl.ds(start + p * rows, rows)]
                piece[...] = x[p * rows:(p + 1) * rows]
                out_copy(piece, pro_rows + i * loop_rows + start + p * rows).start()
        return carry

    lax.fori_loop(0, n_iter, body, 0)
    pltpu.make_async_copy(o_hbm, o_hbm, out_sem).wait()


@jax.jit
def pallas_standalone__cross_network_dcn_v2__recsys_kernel(
    x0: jax.Array,
    U: jax.Array,
    V: jax.Array,
    bs: jax.Array,
):
    batch, dim = x0.shape
    n_layers = U.shape[0]
    chunk_rows = [sum(tiles) for tiles in _PROLOGUE]
    loop_rows = sum(_LOOP_TILES)
    n_iter, leftover = divmod(batch - sum(chunk_rows), loop_rows)
    assert n_iter >= 1 and leftover == 0 and n_layers >= 2

    hbm = pl.BlockSpec(memory_space=pl.ANY)
    return pl.pallas_call(
        _dcn_kernel,
        in_specs=[hbm] * 4,
        out_specs=hbm,
        out_shape=jax.ShapeDtypeStruct((batch, dim), x0.dtype),
        scratch_shapes=(
            [pltpu.VMEM((n_iter, loop_rows, dim), x0.dtype)]
            + [pltpu.VMEM((rows, dim), x0.dtype) for rows in chunk_rows]
            + [pltpu.VMEM(U.shape[1:], U.dtype)] * n_layers
            + [pltpu.VMEM(V.shape[1:], V.dtype)] * n_layers
            + [pltpu.VMEM(bs.shape, bs.dtype),
               pltpu.SemaphoreType.DMA((4,)),
               pltpu.SemaphoreType.DMA(())]
        ),
        compiler_params=pltpu.CompilerParams(vmem_limit_bytes=48 * 2**20),
    )(x0, U, V, bs)
```

```python
import jax
import jax.numpy as jnp
from jax import lax
import jax.experimental.pallas as pl
import jax.experimental.pallas.tpu as pltpu

_PROLOGUE = ((256,), (512,), (512, 512, 528))
_LOOP_TILES = (528,) * 5 + (512,) * 3 + (256, 256)
_LAST_SPLIT = 4

_NT = (((1,), (1,)), ((), ()))


def _offsets(sizes):
    out, start = [], 0
    for size in sizes:
        out.append((start, size))
        start += size
    return out


def _dcn_kernel(x_hbm, u_hbm, v_hbm, b_hbm, o_hbm, x_loop, *scratch):
    n_layers = u_hbm.shape[0]
    n_iter, loop_rows, _ = x_loop.shape
    n_pro = len(_PROLOGUE)
    chunks = _offsets([sum(tiles) for tiles in _PROLOGUE])
    pro_rows = sum(size for _, size in chunks)

    x_pro = scratch[:n_pro]
    u_buf = scratch[n_pro:n_pro + n_layers]
    v_buf = scratch[n_pro + n_layers:n_pro + 2 * n_layers]
    b_buf, in_sem, out_sem = scratch[n_pro + 2 * n_layers:]

    def pro_copy(c):
        start, size = chunks[c]
        sem = in_sem.at[0 if c == 0 else n_layers + c % 2]
        return pltpu.make_async_copy(x_hbm.at[pl.ds(start, size)], x_pro[c], sem)

    def loop_copy(i):
        src = x_hbm.at[pl.ds(pro_rows + i * loop_rows, loop_rows)]
        sem = in_sem.at[n_layers + (n_pro + i) % 2]
        return pltpu.make_async_copy(src, x_loop.at[i], sem)

    def weight_copies(l):
        sem = in_sem.at[l]
        return [pltpu.make_async_copy(v_hbm.at[l], v_buf[l], sem),
                pltpu.make_async_copy(u_hbm.at[l], u_buf[l], sem)]

    def out_copy(src, start):
        return pltpu.make_async_copy(src, o_hbm.at[pl.ds(start, src.shape[0])], out_sem)

    def layer(l, x, x0_f32):
        h = lax.dot_general(x, v_buf[l][...], _NT, preferred_element_type=jnp.float32)
        h = lax.dot_general(h.astype(x.dtype), u_buf[l][...], _NT,
                            preferred_element_type=jnp.float32)
        bias = b_buf[l:l + 1, :].astype(jnp.float32)
        return (x0_f32 * (h + bias) + x.astype(jnp.float32)).astype(x.dtype)

    first = weight_copies(0) + [pro_copy(0),
                                pltpu.make_async_copy(b_hbm, b_buf, in_sem.at[0])]
    for copy in first + weight_copies(1):
        copy.start()
    for l in range(2, n_layers):
        for copy in weight_copies(l):
            copy.start(priority=1)
    pro_copy(1).start(priority=1)

    pending = []
    for c, tiles in enumerate(_PROLOGUE):
        if c == 0:
            for copy in first:
                copy.wait()
        else:
            pro_copy(c).wait()
        if c == n_pro - 2:
            loop_copy(0).start(priority=1)
        for start, size in _offsets(tiles):
            tile = x_pro[c].at[pl.ds(start, size)]
            x = tile[...]
            x0_f32 = x.astype(jnp.float32)
            for l in range(n_layers):
                if c == 0 and start == 0 and l > 0:
                    for copy in weight_copies(l):
                        copy.wait()
                    if l == 1:
                        pro_copy(2).start(priority=1)
                x = layer(l, x, x0_f32)
            tile[...] = x
            pending.append(out_copy(tile, chunks[c][0] + start))

    def body(i, carry):
        loop_copy(i).wait()

        @pl.when(i + 1 < n_iter)
        def _():
            loop_copy(i + 1).start(priority=1)

        @pl.when(i == 0)
        def _():
            for copy in pending:
                copy.start()

        for k, (start, size) in enumerate(_offsets(_LOOP_TILES)):
            x = x_loop[i, pl.ds(start, size), :]
            x0_f32 = x.astype(jnp.float32)
            for l in range(n_layers):
                x = layer(l, x, x0_f32)
            pieces = _LAST_SPLIT if k == len(_LOOP_TILES) - 1 else 1
            rows = size // pieces
            for p in range(pieces):
                piece = x_loop.at[i, pl.ds(start + p * rows, rows)]
                piece[...] = x[p * rows:(p + 1) * rows]
                out_copy(piece, pro_rows + i * loop_rows + start + p * rows).start()
        return carry

    lax.fori_loop(0, n_iter, body, 0)
    pltpu.make_async_copy(o_hbm, o_hbm, out_sem).wait()


@jax.jit
def pallas_standalone__cross_network_dcn_v2__recsys_kernel(
    x0: jax.Array,
    U: jax.Array,
    V: jax.Array,
    bs: jax.Array,
):
    batch, dim = x0.shape
    n_layers = U.shape[0]
    chunk_rows = [sum(tiles) for tiles in _PROLOGUE]
    loop_rows = sum(_LOOP_TILES)
    n_iter, leftover = divmod(batch - sum(chunk_rows), loop_rows)
    assert n_iter >= 1 and leftover == 0 and n_layers >= 2 and len(_PROLOGUE) == 3

    hbm = pl.BlockSpec(memory_space=pl.ANY)
    return pl.pallas_call(
        _dcn_kernel,
        in_specs=[hbm] * 4,
        out_specs=hbm,
        out_shape=jax.ShapeDtypeStruct((batch, dim), x0.dtype),
        scratch_shapes=(
            [pltpu.VMEM((n_iter, loop_rows, dim), x0.dtype)]
            + [pltpu.VMEM((rows, dim), x0.dtype) for rows in chunk_rows]
            + [pltpu.VMEM(U.shape[1:], U.dtype)] * n_layers
            + [pltpu.VMEM(V.shape[1:], V.dtype)] * n_layers
            + [pltpu.VMEM(bs.shape, bs.dtype),
               pltpu.SemaphoreType.DMA((n_layers + 2,)),
               pltpu.SemaphoreType.DMA(())]
        ),
        compiler_params=pltpu.CompilerParams(vmem_limit_bytes=48 * 2**20,
                                             disable_bounds_checks=True),
    )(x0, U, V, bs)
```

```python
import jax
import jax.numpy as jnp
from jax import lax
import jax.experimental.pallas as pl
import jax.experimental.pallas.tpu as pltpu

_PROLOGUE = ((256,), (512,), (512, 512, 528))
_LOOP_TILES = (528,) * 5 + (512,) * 3 + (256, 256)
_LAST_SPLIT = 8

_NT = (((1,), (1,)), ((), ()))


def _offsets(sizes):
    out, start = [], 0
    for size in sizes:
        out.append((start, size))
        start += size
    return out


def _dcn_kernel(x_hbm, u_hbm, v_hbm, b_hbm, o_hbm, x_loop, *scratch):
    n_layers = u_hbm.shape[0]
    n_iter, loop_rows, _ = x_loop.shape
    n_pro = len(_PROLOGUE)
    chunks = _offsets([sum(tiles) for tiles in _PROLOGUE])
    pro_rows = sum(size for _, size in chunks)

    x_pro = scratch[:n_pro]
    u_buf = scratch[n_pro:n_pro + n_layers]
    v_buf = scratch[n_pro + n_layers:n_pro + 2 * n_layers]
    v0t_buf, b_buf, in_sem, out_sem = scratch[n_pro + 2 * n_layers:]

    def pro_copy(c):
        start, size = chunks[c]
        sem = in_sem.at[0 if c == 0 else n_layers + c % 2]
        return pltpu.make_async_copy(x_hbm.at[pl.ds(start, size)], x_pro[c], sem)

    def loop_copy(i):
        src = x_hbm.at[pl.ds(pro_rows + i * loop_rows, loop_rows)]
        sem = in_sem.at[n_layers + (n_pro + i) % 2]
        return pltpu.make_async_copy(src, x_loop.at[i], sem)

    def weight_copies(l):
        sem = in_sem.at[l]
        return [pltpu.make_async_copy(v_hbm.at[l], v_buf[l], sem),
                pltpu.make_async_copy(u_hbm.at[l], u_buf[l], sem)]

    def out_copy(src, start):
        return pltpu.make_async_copy(src, o_hbm.at[pl.ds(start, src.shape[0])], out_sem)

    def layer(l, x, x0_f32, first_tile=False):
        if l == 0 and not first_tile:
            h = jnp.dot(x, v0t_buf[...], preferred_element_type=jnp.float32)
        else:
            h = lax.dot_general(x, v_buf[l][...], _NT,
                                preferred_element_type=jnp.float32)
        h = lax.dot_general(h.astype(x.dtype), u_buf[l][...], _NT,
                            preferred_element_type=jnp.float32)
        bias = b_buf[l:l + 1, :].astype(jnp.float32)
        return (x0_f32 * (h + bias) + x.astype(jnp.float32)).astype(x.dtype)

    first = weight_copies(0) + [pro_copy(0),
                                pltpu.make_async_copy(b_hbm, b_buf, in_sem.at[0])]
    for copy in first + weight_copies(1):
        copy.start()
    for l in range(2, n_layers):
        for copy in weight_copies(l):
            copy.start(priority=1)
    pro_copy(1).start(priority=1)

    pending = []
    for c, tiles in enumerate(_PROLOGUE):
        if c == 0:
            for copy in first:
                copy.wait()
        else:
            pro_copy(c).wait()
        if c == n_pro - 2:
            loop_copy(0).start(priority=1)
        for start, size in _offsets(tiles):
            first_tile = c == 0 and start == 0
            tile = x_pro[c].at[pl.ds(start, size)]
            x = tile[...]
            x0_f32 = x.astype(jnp.float32)
            for l in range(n_layers):
                if first_tile and l > 0:
                    for copy in weight_copies(l):
                        copy.wait()
                    if l == 1:
                        pro_copy(2).start(priority=1)
                if first_tile and l == n_layers - 1:
                    v0t_buf[...] = v_buf[0][...].T
                x = layer(l, x, x0_f32, first_tile)
            tile[...] = x
            pending.append(out_copy(tile, chunks[c][0] + start))

    def body(i, carry):
        loop_copy(i).wait()

        @pl.when(i + 1 < n_iter)
        def _():
            loop_copy(i + 1).start(priority=1)

        @pl.when(i == 0)
        def _():
            for copy in pending:
                copy.start()

        for k, (start, size) in enumerate(_offsets(_LOOP_TILES)):
            x = x_loop[i, pl.ds(start, size), :]
            x0_f32 = x.astype(jnp.float32)
            for l in range(n_layers):
                x = layer(l, x, x0_f32)
            pieces = _LAST_SPLIT if k == len(_LOOP_TILES) - 1 else 1
            rows = size // pieces
            for p in range(pieces):
                piece = x_loop.at[i, pl.ds(start + p * rows, rows)]
                piece[...] = x[p * rows:(p + 1) * rows]
                out_copy(piece, pro_rows + i * loop_rows + start + p * rows).start()
        return carry

    lax.fori_loop(0, n_iter, body, 0)
    pltpu.make_async_copy(o_hbm, o_hbm, out_sem).wait()


@jax.jit
def pallas_standalone__cross_network_dcn_v2__recsys_kernel(
    x0: jax.Array,
    U: jax.Array,
    V: jax.Array,
    bs: jax.Array,
):
    batch, dim = x0.shape
    n_layers, rank, _ = V.shape
    chunk_rows = [sum(tiles) for tiles in _PROLOGUE]
    loop_rows = sum(_LOOP_TILES)
    n_iter, leftover = divmod(batch - sum(chunk_rows), loop_rows)
    assert n_iter >= 1 and leftover == 0 and n_layers >= 2 and len(_PROLOGUE) == 3

    hbm = pl.BlockSpec(memory_space=pl.ANY)
    return pl.pallas_call(
        _dcn_kernel,
        in_specs=[hbm] * 4,
        out_specs=hbm,
        out_shape=jax.ShapeDtypeStruct((batch, dim), x0.dtype),
        scratch_shapes=(
            [pltpu.VMEM((n_iter, loop_rows, dim), x0.dtype)]
            + [pltpu.VMEM((rows, dim), x0.dtype) for rows in chunk_rows]
            + [pltpu.VMEM(U.shape[1:], U.dtype)] * n_layers
            + [pltpu.VMEM(V.shape[1:], V.dtype)] * n_layers
            + [pltpu.VMEM((dim, rank), V.dtype),
               pltpu.VMEM(bs.shape, bs.dtype),
               pltpu.SemaphoreType.DMA((n_layers + 2,)),
               pltpu.SemaphoreType.DMA(())]
        ),
        compiler_params=pltpu.CompilerParams(vmem_limit_bytes=48 * 2**20,
                                             disable_bounds_checks=True),
    )(x0, U, V, bs)
```
